```python
import jax
import jax.numpy as jnp

def _softmax(x, axis=-1):
    return jax.nn.softmax(x, axis=axis)
def _gelu(x):
    return jax.nn.gelu(x, approximate=True)
def _silu(x):
    return jax.nn.silu(x)
def _sigmoid(x):
    return jax.nn.sigmoid(x)
def _layernorm(x, axis=-1, eps=1e-5):
    m = jnp.mean(x, axis=axis, keepdims=True)
    v = jnp.var(x, axis=axis, keepdims=True)
    return (x - m) / jnp.sqrt(v + eps)
def _scatter_add(tgt, idx, src, axis=0):
    return tgt.at[idx].add(src)
def _segment_sum(src, seg, n):
    return jax.ops.segment_sum(src, seg, n)
class _Rng:
    def __init__(self, key):
        self._k = key
    def _next(self):
        self._k, sub = jax.random.split(self._k)
        return sub
    def normal(self, shape):
        return jax.random.normal(self._next(), shape, dtype=jnp.bfloat16)
    def randint(self, lo, hi, shape):
        return jax.random.randint(self._next(), shape, lo, hi, dtype=jnp.int32)
    def uniform(self, shape, lo=0.0, hi=1.0):
        return jax.random.uniform(self._next(), shape, jnp.bfloat16, lo, hi)
    def permutation(self, n):
        return jax.random.permutation(self._next(), n)


kernel_name = 'concat_heads__ssm_conv_h3__linear_attn_block__prompt'

def setup_inputs():
    _rng = _Rng(jax.random.key(int.from_bytes(__import__("os").urandom(4), "little")))
    _w = (lambda a: (lambda t: t.astype(jnp.bfloat16) if jnp.issubdtype(t.dtype, jnp.floating) else t)(jnp.asarray(a)))
    def _A_setup():
        B, S, D = 1, 2048, 1024
        ks = 4
        return {
            "q": _w((lambda *s: _rng.normal(s) * 0.05)(B, S, D)),
            "k": _w((lambda *s: _rng.normal(s) * 0.05)(B, S, D)),
            "v": _w((lambda *s: _rng.normal(s) * 0.05)(B, S, D)),
            "shift_k": _w((lambda *s: _rng.normal(s) * 0.05)(D, ks) * 0.5),
            "ssm_k": _w((lambda *s: _rng.normal(s) * 0.05)(D, S) * (1.0 / S ** 0.5)),
            "ssm_D": _w((lambda *s: _rng.normal(s) * 0.05)(D)),
        }
    _A_in = _A_setup()

    def _B_setup():
        B, S, D = 1, 2048, 1024
        return {
            "x": _w((lambda *s: _rng.normal(s) * 0.05)(B, S, D)),
            "wqkv": _w((lambda *s: _rng.normal(s) * 0.05)(D, 3 * D)),
            "wo": _w((lambda *s: _rng.normal(s) * 0.05)(D, D)),
        }
    _B_in = _B_setup()

    return {
        "A_q": _A_in["q"],
        "A_k": _A_in["k"],
        "A_v": _A_in["v"],
        "A_shift_k": _A_in["shift_k"],
        "A_ssm_k": _A_in["ssm_k"],
        "A_ssm_D": _A_in["ssm_D"],
        "B_x": _B_in["x"],
        "B_wqkv": _B_in["wqkv"],
        "B_wo": _B_in["wo"],
    }

def reference(A_q, A_k, A_v, A_shift_k, A_ssm_k, A_ssm_D, B_x, B_wqkv, B_wo):
    def _A_ref(q, k, v, shift_k, ssm_k, ssm_D):
        B, S, D = q.shape
        ks = shift_k.shape[-1]
        k_pad = jnp.pad(k, ((0, 0), (ks - 1, 0), (0, 0)))
        k_shift = jnp.zeros_like(k)
        for t in range(ks):
            k_shift = k_shift + k_pad[:, t:t + S, :] * shift_k[:, ks - 1 - t][None, None, :]
        kv = k_shift * v
        L = 2 * S
        kv_pad = jnp.pad(kv, ((0, 0), (0, S), (0, 0)))
        kf_pad = jnp.pad(ssm_k, ((0, 0), (0, S)))
        kv_f = (lambda x, axes=(-2,-1): jnp.fft.rfft2(x.astype(jnp.float32), axes=axes))(kv_pad[:, None, :, :], axes=(1, 2))
        kf_f = (lambda x, axes=(-2,-1): jnp.fft.rfft2(x.astype(jnp.float32), axes=axes))(kf_pad[:, None, :], axes=(1, 2))
        kf_f = (lambda x, *d: x.transpose(*d))(kf_f, 1, 2, 0)
        y_f = kv_f * kf_f[None, :, :, :]
        y = (lambda x, s, axes=(-2,-1): jnp.fft.irfft2(x, s=s, axes=axes).astype(jnp.bfloat16))(y_f, (1, L), axes=(1, 2))[:, 0, :S, :]
        y = y + kv * ssm_D[None, None, :]
        return q * y

    def _B_ref(x, wqkv, wo):
        B, S, D = x.shape
        H = 32; Dh = D // H
        qkv = (lambda x, *d: x.transpose(*d))((x @ wqkv).reshape(B, S, 3, H, Dh), 2, 0, 3, 1, 4)
        q, k, v = qkv[0], qkv[1], qkv[2]
        phi = lambda t: jnp.where(t > 0, t + 1, jnp.exp(t)) + 1e-6
        pq, pk = phi(q), phi(k)
        kv = jnp.einsum("bhsd,bhse->bhde", pk, v)
        z = jnp.einsum("bhsd->bhd", pk)
        num = jnp.einsum("bhqd,bhde->bhqe", pq, kv)
        den = jnp.einsum("bhqd,bhd->bhq", pq, z)[..., None] + 1e-6
        o = num / den
        return (lambda x, *d: x.transpose(*d))(o, 0, 2, 1, 3).reshape(B, S, D) @ wo

    a = _A_ref(A_q, A_k, A_v, A_shift_k, A_ssm_k, A_ssm_D)
    b = _B_ref(B_x, B_wqkv, B_wo)
    return jnp.concatenate([a, b], axis=-1)
```

```python
import jax, jax.numpy as jnp, numpy as np
import jax.experimental.pallas as pl
import jax.experimental.pallas.tpu as pltpu
S, D = 2048, 1024
f32, bf16 = jnp.float32, jnp.bfloat16
P = 2; L = S // P; N = 2 * L; N2 = 8; N1 = 128
RT = 16

def _consts():
    k1 = np.concatenate([np.arange(0, 128, 2), np.arange(1, 128, 2)])
    n1 = np.arange(N1)
    F = np.zeros((N2, 256, 128), np.float32); G = np.zeros((N2, 128, 256), np.float32)
    for n2 in range(N2):
        ang = -2 * np.pi * (((2 * k1[:, None] + 1) * (N2 * n1[None, :] + n2)) % (2 * N)) / (2 * N)
        F[n2, :128] = np.cos(ang); F[n2, 128:] = np.sin(ang)
        G[n2, :, :128] = (2.0 / N) * np.cos(ang).T; G[n2, :, 128:] = (2.0 / N) * np.sin(ang).T
    return F, G

def _tw(z, e, sgn):
    a, b = z
    e = (e * sgn) % 8
    c = float(np.sqrt(0.5))
    if e == 0: return a, b
    if e == 2: return -b, a
    if e == 6: return b, -a
    if e == 4: return -a, -b
    if e == 1: return (a - b) * c, (a + b) * c
    if e == 7: return (a + b) * c, (b - a) * c
    if e == 3: return (a + b) * (-c), (a - b) * c
    if e == 5: return (b - a) * c, (a + b) * (-c)

def _bfly(u, z, e, sgn):
    (ur, ui), (a, b) = u, z
    if e == 0:
        return (ur + a, ui + b), (ur - a, ui - b)
    if e == 2:
        if sgn > 0:
            return (ur - b, ui + a), (ur + b, ui - a)
        return (ur + b, ui - a), (ur - b, ui + a)
    tr, ti = _tw(z, e, sgn)
    return (ur + tr, ui + ti), (ur - tr, ui - ti)

def _fft(x, sgn):
    n = len(x)
    if n == 1: return x
    e = _fft(x[0::2], sgn); o = _fft(x[1::2], sgn)
    out = [None] * n
    for k in range(n // 2):
        out[k], out[k + n // 2] = _bfly(e[k], o[k], k * (8 // n), sgn)
    return out

def _cmul(x, h):
    return x[0] * h[0] - x[1] * h[1], x[0] * h[1] + x[1] * h[0]


R = 256
NB = S // R

def phi(t):
    return jnp.where(t > 0, t + 1.0, jnp.exp(t)) + 1e-6

def a_stage1(k_ref, v_ref, h_ref, sk_ref, d_ref, f_ref, ks_ref, kv_ref, ht_ref, s1_ref):
    w = sk_ref[...].astype(f32)
    ks_ref[0:8, :] = jnp.zeros((8, 128), f32)
    ks_ref[8:, :] = k_ref[...].astype(f32)
    ksh = ks_ref[pl.ds(8, S), :] * w[0:1]
    for t in range(1, 4):
        ksh = ksh + ks_ref[pl.ds(8 - t, S), :] * w[t:t + 1]
    kv_ref[...] = ksh * v_ref[...].astype(f32)
    ht_ref[...] = h_ref[...].astype(f32).T
    ht_ref[0:1, :] = ht_ref[0:1, :] + d_ref[...].astype(f32).reshape(1, 128)
    for a, src in enumerate((kv_ref, ht_ref)):
        for p in range(P):
            for n2 in range(N2):
                xs = src[pl.ds(p * L + n2, N1, stride=N2), :].astype(bf16)
                s1_ref[a, p, n2] = jnp.dot(f_ref[n2], xs, preferred_element_type=f32)

def a_stage2(s1_ref, y1_ref):
    for r in range(0, 128, RT):
        def ld(a, p):
            return _fft([(s1_ref[a, p, n2, r:r + RT, :], s1_ref[a, p, n2, 128 + r:128 + r + RT, :]) for n2 in range(N2)], -1)
        X0 = ld(0, 0); H0 = ld(1, 0); H1 = ld(1, 1)
        if r < 64:
            G = [(g[0] - h[1], g[1] + h[0]) for g, h in zip(H1, H0)]
        else:
            G = [(g[0] + h[1], g[1] - h[0]) for g, h in zip(H1, H0)]
        Y1 = [_cmul(x, g) for x, g in zip(X0, G)]
        Y0 = [_cmul(x, h) for x, h in zip(X0, H0)]
        y0 = _fft(Y0, 1)
        for n2 in range(N2):
            y1_ref[0, n2, r:r + RT, :] = y0[n2][0].astype(bf16)
            y1_ref[0, n2, 128 + r:128 + r + RT, :] = y0[n2][1].astype(bf16)
        X1 = ld(0, 1)
        Y1 = [(y[0] + m[0], y[1] + m[1]) for y, m in zip(Y1, [_cmul(x, h) for x, h in zip(X1, H0)])]
        y1 = _fft(Y1, 1)
        for n2 in range(N2):
            y1_ref[1, n2, r:r + RT, :] = y1[n2][0].astype(bf16)
            y1_ref[1, n2, 128 + r:128 + r + RT, :] = y1[n2][1].astype(bf16)

def a_inv(q_ref, g_ref, y1_ref, ys_ref, o_ref):
    for p in range(P):
        for n2 in range(N2):
            ys_ref[pl.ds(p * L + n2, N1, stride=N2), :] = jnp.dot(g_ref[n2], y1_ref[p, n2], preferred_element_type=f32)
    o_ref[...] = (q_ref[...].astype(f32) * ys_ref[...]).astype(bf16)

def kern(q_ref, k_ref, v_ref, h_ref, sk_ref, d_ref, f_ref, x_ref, g_hbm, w_hbm, wo_hbm, o_hbm,
         ks_ref, kv_ref, ht_ref, s1_ref, y1_ref, g_ref, w_ref, wo_ref, kvacc_ref, z_ref, m_ref, zb_ref, pk_ref, oa_ref, ob_ref, wsem, osem):
    i = pl.program_id(0)
    def wcopy(j):
        return pltpu.make_async_copy(w_hbm.at[:, j * D:(j + 1) * D], w_ref.at[j], wsem.at[j])
    wocopy = pltpu.make_async_copy(wo_hbm, wo_ref, wsem.at[3])
    gcopy = pltpu.make_async_copy(g_hbm, g_ref, wsem.at[4])
    def acopy(j, slot):
        return pltpu.make_async_copy(oa_ref.at[slot], o_hbm.at[:, pl.ds(pl.multiple_of(j * 128, 128), 128)], osem.at[slot])
    def bcopy(j, slot):
        return pltpu.make_async_copy(ob_ref.at[slot], o_hbm.at[pl.ds(pl.multiple_of(j * R, R), R), D:2 * D], osem.at[2 + slot])

    @pl.when(i == 0)
    def _():
        wcopy(1).start(); wcopy(2).start()
        kvacc_ref[...] = jnp.zeros_like(kvacc_ref)
        z_ref[...] = jnp.zeros_like(z_ref)

    @pl.when(i < NB)
    def _():
        a_stage1(k_ref, v_ref, h_ref, sk_ref, d_ref, f_ref, ks_ref, kv_ref, ht_ref, s1_ref)
        a_stage2(s1_ref, y1_ref.at[i])

    @pl.when(i == 0)
    def _():
        wcopy(1).wait()

    @pl.when(i < NB)
    def _():
        k = jnp.dot(x_ref[...], w_ref[1], preferred_element_type=f32)
        pk = phi(k)
        z_ref[...] += jnp.sum(pk.reshape(R // 8, 8, D), axis=0)
        pk_ref[...] = pk.astype(bf16)

    @pl.when(i == 0)
    def _():
        wcopy(2).wait()
        wcopy(0).start(); wocopy.start(); gcopy.start()

    @pl.when(i < NB)
    def _():
        v = jnp.dot(x_ref[...], w_ref[2], preferred_element_type=f32).astype(bf16)
        for g in range(8):
            kvacc_ref[g] += jax.lax.dot_general(pk_ref[:, g*128:(g+1)*128], v[:, g*128:(g+1)*128], (((0,), (0,)), ((), ())), preferred_element_type=f32)

    @pl.when(i == NB)
    def _():
        wcopy(0).wait(); wocopy.wait(); gcopy.wait()
        r = jax.lax.broadcasted_iota(jnp.int32, (128, 128), 0) // 32
        c = jax.lax.broadcasted_iota(jnp.int32, (128, 128), 1) // 32
        mask = r == c
        z = jnp.sum(z_ref[...], axis=0, keepdims=True)
        for g in range(8):
            kvm = jnp.where(mask, kvacc_ref[g], 0.0).astype(bf16)
            m_ref[g*128:(g+1)*128, :] = jnp.dot(kvm, wo_ref[g*128:(g+1)*128, :], preferred_element_type=f32).astype(bf16)
            zc = jnp.broadcast_to(z[:, g*128:(g+1)*128], (128, 128)).T
            zb_ref[g] = jnp.where(mask, zc, 0.0).astype(bf16)

    j = i - NB
    slot = j % 2
    @pl.when(j >= 2)
    def _():
        acopy(j - 2, slot).wait(); bcopy(j - 2, slot).wait()

    @pl.when(i >= NB)
    def _():
        pns = []
        for c in range(2):
            q = jnp.dot(x_ref[...], w_ref[0, :, c*512:(c+1)*512], preferred_element_type=f32)
            pq = phi(q)
            pqb = pq.astype(bf16)
            for g in range(4):
                den = jnp.dot(pqb[:, g*128:(g+1)*128], zb_ref[c*4+g], preferred_element_type=f32) + 1e-6
                pns.append((pq[:, g*128:(g+1)*128] * pl.reciprocal(den, approx=True)).astype(bf16))
        a_inv(q_ref, g_ref, y1_ref.at[j], ht_ref, oa_ref.at[slot])
        pn = jnp.concatenate(pns, axis=1)
        ob_ref[slot] = jnp.dot(pn, m_ref[...], preferred_element_type=f32).astype(bf16)
        acopy(j, slot).start(); bcopy(j, slot).start()

    @pl.when(j == NB - 1)
    def _():
        acopy(j - 1, 1 - slot).wait(); bcopy(j - 1, 1 - slot).wait()
        acopy(j, slot).wait(); bcopy(j, slot).wait()

def pallas_concat_heads__ssm_conv_h3__linear_attn_block__prompt_kernel(A_q, A_k, A_v, A_shift_k, A_ssm_k, A_ssm_D, B_x, B_wqkv, B_wo):
    F, G = _consts()
    fi = lambda i: jnp.minimum(i, NB - 1)
    cb = pl.BlockSpec((S, 128), lambda i: (0, fi(i)))
    anys = pl.BlockSpec(memory_space=pl.ANY)
    out = pl.pallas_call(kern, grid=(2 * NB,),
        in_specs=[pl.BlockSpec((S, 128), lambda i: (0, jnp.maximum(i - NB, 0))), cb, cb,
                  pl.BlockSpec((128, S), lambda i: (fi(i), 0)), pl.BlockSpec((4, 128), lambda i: (0, fi(i))),
                  pl.BlockSpec((None,1,128), lambda i: (fi(i),0,0)),
                  pl.BlockSpec((N2, 256, 128), lambda i: (0, 0, 0)),
                  pl.BlockSpec((R, D), lambda i: (i % NB, 0)), anys, anys, anys],
        out_specs=anys,
        out_shape=jax.ShapeDtypeStruct((S, 2*D), bf16),
        scratch_shapes=[pltpu.VMEM((S + 8, 128), f32), pltpu.VMEM((S, 128), f32), pltpu.VMEM((S, 128), f32),
                        pltpu.VMEM((2, P, N2, 256, 128), f32), pltpu.VMEM((8, P, N2, 256, 128), bf16),
                        pltpu.VMEM((N2, 128, 256), bf16), pltpu.VMEM((3, D, D), bf16), pltpu.VMEM((D, D), bf16),
                        pltpu.VMEM((8, 128, 128), f32), pltpu.VMEM((8, D), f32), pltpu.VMEM((D, D), bf16), pltpu.VMEM((8, 128, 128), bf16),
                        pltpu.VMEM((R, D), bf16), pltpu.VMEM((2, S, 128), bf16), pltpu.VMEM((2, R, D), bf16),
                        pltpu.SemaphoreType.DMA((5,)), pltpu.SemaphoreType.DMA((4,))],
        compiler_params=pltpu.CompilerParams(dimension_semantics=("arbitrary",), vmem_limit_bytes=100*1024*1024),
    )(A_q.reshape(S, D), A_k.reshape(S, D), A_v.reshape(S, D), A_ssm_k, A_shift_k.T, A_ssm_D.reshape(8,1,128), F.astype(bf16), B_x.reshape(S, D), G.astype(bf16), B_wqkv, B_wo)
    return out.reshape(1, S, 2*D)
```
